```python
import os as _os
_os.environ.setdefault('JAX_PLATFORMS', 'cpu')
import jax
import jax.numpy as jnp

def _softmax(x, axis=-1):
    return jax.nn.softmax(x, axis=axis)

def _gelu(x):
    return jax.nn.gelu(x, approximate=True)

def _silu(x):
    return jax.nn.silu(x)

def _sigmoid(x):
    return jax.nn.sigmoid(x)

def _layernorm(x, axis=-1, eps=1e-05):
    m = jnp.mean(x, axis=axis, keepdims=True)
    v = jnp.var(x, axis=axis, keepdims=True)
    return (x - m) / jnp.sqrt(v + eps)

def _scatter_add(tgt, idx, src, axis=0):
    return tgt.at[idx].add(src)

def _segment_sum(src, seg, n):
    return jax.ops.segment_sum(src, seg, n)

class _Rng:

    def __init__(self, key):
        self._k = key

    def _next(self):
        self._k, sub = jax.random.split(self._k)
        return sub

    def normal(self, shape):
        return jax.random.normal(self._next(), shape, dtype=jnp.bfloat16)

    def randint(self, lo, hi, shape):
        return jax.random.randint(self._next(), shape, lo, hi, dtype=jnp.int32)

    def uniform(self, shape, lo=0.0, hi=1.0):
        return jax.random.uniform(self._next(), shape, jnp.bfloat16, lo, hi)

    def permutation(self, n):
        return jax.random.permutation(self._next(), n)
kernel_name = 'standalone__conformer_family_zipformer__speech'

def setup_inputs():
    _rng = _Rng(jax.random.key(int.from_bytes(__import__("os").urandom(4), "little")))
    _w = lambda a: (lambda t: t.astype(jnp.bfloat16) if jnp.issubdtype(t.dtype, jnp.floating) else t)(jnp.asarray(a))
    B, T, D, K, H = (2, 4000, 144, 3, 4)
    sc = 0.1
    return {'x': _w((lambda *s: _rng.normal(s) * 0.8)(B, T, D)), 'w_ff1a': _w((lambda *s: _rng.normal(s) * 0.8)(D, 4 * D) * sc), 'w_ff1b': _w((lambda *s: _rng.normal(s) * 0.8)(4 * D, D) * sc), 'w_qkv': _w((lambda *s: _rng.normal(s) * 0.8)(D, 3 * D) * sc), 'w_o': _w((lambda *s: _rng.normal(s) * 1.6)(D, D) * sc), 'w_pw1': _w((lambda *s: _rng.normal(s) * 1.6)(D, 2 * D) * sc), 'dw': _w((lambda *s: _rng.normal(s) * 0.4)(K, D)), 'w_pw2': _w((lambda *s: _rng.normal(s) * 0.4)(D, D) * sc), 'w_ff2a': _w((lambda *s: _rng.normal(s) * 0.8)(D, 4 * D) * sc), 'w_ff2b': _w((lambda *s: _rng.normal(s) * 0.8)(4 * D, D) * sc)}

def reference(x, w_ff1a, w_ff1b, w_qkv, w_o, w_pw1, dw, w_pw2, w_ff2a, w_ff2b):
    B, T, D = x.shape
    K = dw.shape[0]
    H = 4
    Dh = D // H
    h = _layernorm(x, axis=-1)
    h = _silu(h @ w_ff1a) @ w_ff1b
    x = x + 0.5 * h
    h = _layernorm(x, axis=-1)
    qkv = h @ w_qkv
    q = (lambda x, *d: x.transpose(*d))(qkv[..., :D].reshape(B, T, H, Dh), 0, 2, 1, 3)
    k = (lambda x, *d: x.transpose(*d))(qkv[..., D:2 * D].reshape(B, T, H, Dh), 0, 2, 1, 3)
    v = (lambda x, *d: x.transpose(*d))(qkv[..., 2 * D:].reshape(B, T, H, Dh), 0, 2, 1, 3)
    scale = Dh ** (-0.5)
    scores = jnp.einsum('bhqd,bhkd->bhqk', q, k) * scale
    p = _softmax(scores, axis=-1)
    att = jnp.einsum('bhqk,bhkd->bhqd', p, v)
    att = (lambda x, *d: x.transpose(*d))(att, 0, 2, 1, 3).reshape(B, T, D)
    x = x + att @ w_o
    h = _layernorm(x, axis=-1)
    h = h @ w_pw1
    a, b = (h[..., :D].copy(), h[..., D:].copy())
    h = a * _sigmoid(b)
    pad = K // 2
    hp = jnp.pad(h, ((0, 0), (pad, pad), (0, 0)))
    c = jnp.zeros_like(h)
    for i in range(K):
        c = c + hp[:, i:i + T, :] * dw[i][None, None, :]
    x = x + _silu(c) @ w_pw2
    h = _layernorm(x, axis=-1)
    h = _silu(h @ w_ff2a) @ w_ff2b
    x = x + 0.5 * h
    return _layernorm(x, axis=-1)
```

```python
import jax
import jax.numpy as jnp
import jax.experimental.pallas as pl
import jax.experimental.pallas.tpu as pltpu

F32 = jnp.float32
BF16 = jnp.bfloat16
U32 = jnp.uint32

B, T, D, H, DH, KW = 2, 4000, 144, 4, 36, 3
FF = 4 * D
TP = 4096
TB = 512
NB = TP // TB
TQ = 512
TK = 1024
RB = 128
VR = 40
HP = 2 * DH
KD = 128
EPS = 1e-5
NEG = -1e30
QSCALE = float(DH ** -0.5 * 1.4426950408889634)
CHUNKS = [(c * TK, min(TK, T - c * TK)) for c in range(-(-T // TK))]
NC = len(CHUNKS)


def _pk(x):
    return pltpu.bitcast(x, U32)


def _upk(x):
    return pltpu.bitcast(x, BF16)


def _dot(a, b):
    return jnp.dot(a, b, preferred_element_type=F32)


def _dot_nt(a, b):
    return jax.lax.dot_general(a, b, (((1,), (1,)), ((), ())), preferred_element_type=F32)


def _ln(x):
    m = jnp.mean(x, axis=0, keepdims=True)
    xc = x - m
    v = jnp.mean(xc * xc, axis=0, keepdims=True)
    return xc * jax.lax.rsqrt(v + EPS)


def _sigmoid(x):
    return 0.5 * jnp.tanh(0.5 * x) + 0.5


def _silu(x):
    h = 0.5 * x
    return h * jnp.tanh(h) + h


def _iota(shape, dim):
    return jax.lax.broadcasted_iota(jnp.int32, shape, dim)


def _sel_t(w, n_out, row_of_col):
    n = w.shape[1]
    r = _iota((n_out, n), 0)
    c = _iota((n_out, n), 1)
    e = jnp.where(r == row_of_col(c), 1.0, 0.0).astype(BF16)
    return _pk(_dot_nt(e, w).astype(BF16))


def _kernel(x_ref, w1a_ref, w1b_ref, wqkv_ref, wo_ref, wp1_ref, dw_ref, wp2_ref, w2a_ref, w2b_ref,
            o_ref,
            w1a_t, w1b_t, wqkv_t, wo_t, wp1_t, wp2_t, w2a_t, w2b_t, dw_t,
            xp_ref, x1_ref, qt_ref, k_ref, vt_ref, acc_ref, g_ref, y_ref, s0, s1):
    ident = lambda c: c

    @pl.when(pl.program_id(0) == 0)
    def _prep():
        w1a_t[...] = _sel_t(w1a_ref[...], FF, ident)
        w1b_t[...] = _sel_t(w1b_ref[...], D, ident)
        w2a_t[...] = _sel_t(w2a_ref[...], FF, ident)
        w2b_t[...] = _sel_t(w2b_ref[...], D, ident)
        wp1_t[...] = _sel_t(wp1_ref[...], 2 * D, ident)
        wp2_t[...] = _sel_t(wp2_ref[...], D, ident)
        wqkv_t[...] = _sel_t(
            wqkv_ref[...], 2 * D + H * VR,
            lambda c: jnp.where(c < 2 * D, c, 2 * D + ((c - 2 * D) // DH) * VR + (c - 2 * D) % DH))
        r = _iota((D, H * VR), 0)
        c = _iota((D, H * VR), 1)
        e = jnp.where((c // VR) * DH + c % VR == r, jnp.where(c % VR < DH, 1.0, 0.0), 0.0).astype(BF16)
        wo_tr = _upk(_sel_t(wo_ref[...], D, ident))
        wo_t[...] = _pk(_dot(wo_tr, e).astype(BF16))
        dwt = _upk(_sel_t(jnp.concatenate([dw_ref[...], jnp.zeros((16 - KW, D), BF16)], axis=0), D, ident))
        dwt = dwt.astype(F32)
        for i in range(KW):
            dw_t[i] = jnp.broadcast_to(dwt[:, i:i + 1], (D, 128))
        g_ref[:, 0:128] = jnp.zeros((D, 128), F32)
        g_ref[:, 128 + TP:] = jnp.zeros((D, 128), F32)

    xp_ref[0:T, :] = x_ref[0]
    xp_ref[T:TP, :] = jnp.zeros((TP - T, D), BF16)

    def ffn(x, wa_t, wb_t):
        h = _ln(x).astype(BF16)
        a = _silu(_dot(_upk(wa_t[...]), h)).astype(BF16)
        return x + 0.5 * _dot(_upk(wb_t[...]), a)

    def phase1(i, carry):
        start = pl.multiple_of(i * TB, TB)
        cols = pl.ds(start, TB)
        xt = xp_ref[cols, :].astype(F32).T
        x1 = ffn(xt, w1a_t, w1b_t)
        x1_ref[:, cols] = x1
        h = _ln(x1).astype(BF16)
        qkv = _dot(_upk(wqkv_t[...]), h)
        row = _iota((HP, TB), 0)
        zpad = jnp.zeros((KD - HP, TB), F32)
        for pair in range(2):
            qp = qkv[pair * HP:(pair + 1) * HP] * QSCALE
            q_lo = jnp.concatenate([jnp.where(row < DH, qp, 0.0), zpad], axis=0)
            q_hi = jnp.concatenate([jnp.where(row >= DH, qp, 0.0), zpad], axis=0)
            qt_ref[2 * pair, :, cols] = _pk(q_lo.astype(BF16))
            qt_ref[2 * pair + 1, :, cols] = _pk(q_hi.astype(BF16))
            kt = jnp.concatenate([qkv[D + pair * HP:D + (pair + 1) * HP], zpad], axis=0)
            k_ref[pair, pl.ds(pl.multiple_of(i * (TB // 2), TB // 2), TB // 2), :] = _pk(kt.T.astype(BF16))
        vrow = _iota((H * VR, TB), 0)
        v = jnp.where(vrow % VR == DH, 1.0, qkv[2 * D:])
        for h_ in range(H):
            vt_ref[h_, :, cols] = v[h_ * VR:(h_ + 1) * VR]
        return carry

    jax.lax.fori_loop(0, NB, phase1, 0)

    S = (s0, s1)
    NU = NB * H

    def unit(u):
        u = jnp.minimum(u, NU - 1)
        return u // H, u % H

    def get_q(u):
        q, h = unit(u)
        return _upk(qt_ref[h, :, pl.ds(pl.multiple_of(q * TQ, TQ), TQ)])

    def sub_a(u, c, r, par, qt, z):
        _, h = unit(u)
        start, size = CHUNKS[c]
        n = min(RB, size - r * RB)
        off = (start + r * RB) // 2
        k = _upk(k_ref[h // 2, off:off + n // 2, :])
        s = _dot(k, qt)
        S[par][pl.ds(pl.multiple_of(z + r * RB, 8), n), :] = s
        return jnp.max(s, axis=0, keepdims=True)

    def nsub(c):
        return -(-CHUNKS[c][1] // RB)

    def att_body(u, mx):
        q, h = unit(u)
        z = (u // NU) * 8
        qs = pl.ds(pl.multiple_of(q * TQ, TQ), TQ)
        m_prev = None
        acc = None
        for c in range(NC):
            par = c % 2
            last = c == NC - 1
            un, cn = (u + 1, 0) if last else (u, c + 1)
            qt = get_q(un)
            if m_prev is None:
                m_new = mx
            else:
                m_new = jnp.maximum(m_prev, mx)
                alpha = jnp.exp2(m_prev - m_new)
            mx = None
            pv = None
            start, size = CHUNKS[c]
            for r in range(max(nsub(c), nsub(cn))):
                if r < nsub(cn):
                    mr = sub_a(un, cn, r, 1 - par, qt, z)
                    mx = mr if mx is None else jnp.maximum(mx, mr)
                if r < nsub(c):
                    n = min(RB, size - r * RB)
                    p = jnp.exp2(S[par][r * RB:r * RB + n, :] - m_new).astype(BF16)
                    vt = vt_ref[h, :, start + r * RB:start + r * RB + n]
                    d = _dot(vt, p)
                    pv = d if pv is None else pv + d
            acc = pv if acc is None else acc * alpha + pv
            m_prev = m_new
        acc_ref[h, :, qs] = acc
        return mx

    qt0 = get_q(0)
    mx0 = None
    for r in range(nsub(0)):
        mr = sub_a(0, 0, r, 0, qt0, 0)
        mx0 = mr if mx0 is None else jnp.maximum(mx0, mr)
    jax.lax.fori_loop(0, NU, att_body, mx0)

    def phase2(i, carry):
        start = pl.multiple_of(i * TB, TB)
        cols = pl.ds(start, TB)
        outs = []
        for h_ in range(H):
            a = acc_ref[h_, :, cols]
            outs.append(a * (1.0 / a[DH:DH + 1, :]))
        o = jnp.concatenate(outs, axis=0).astype(BF16)
        x2 = x1_ref[:, cols] + _dot(_upk(wo_t[...]), o)
        x1_ref[:, cols] = x2
        h = _ln(x2).astype(BF16)
        g = _dot(_upk(wp1_t[...]), h)
        glu = g[:D] * _sigmoid(g[D:])
        tok = start + _iota((D, TB), 1)
        g_ref[:, pl.ds(pl.multiple_of(start + 128, 128), TB)] = jnp.where(tok < T, glu, 0.0)
        return carry

    jax.lax.fori_loop(0, NB, phase2, 0)

    def phase3(i, carry):
        start = pl.multiple_of(i * TB, TB)
        cols = pl.ds(start, TB)
        win = g_ref[:, pl.ds(start, TB + 256)]
        left = pltpu.roll(win, 1, 1)[:, 128:128 + TB]
        right = pltpu.roll(win, TB + 255, 1)[:, 128:128 + TB]
        cur = win[:, 128:128 + TB]
        rep = lambda w: jnp.concatenate([w] * (TB // 128), axis=1)
        c = left * rep(dw_t[0]) + cur * rep(dw_t[1]) + right * rep(dw_t[2])
        x3 = x1_ref[:, cols] + _dot(_upk(wp2_t[...]), _silu(c).astype(BF16))
        x4 = ffn(x3, w2a_t, w2b_t)
        y_ref[cols, :] = _ln(x4).T.astype(BF16)
        return carry

    jax.lax.fori_loop(0, NB, phase3, 0)
    o_ref[0] = y_ref[0:T, :]


@jax.jit
def pallas_standalone__conformer_family_zipformer__speech_kernel(
    x, w_ff1a, w_ff1b, w_qkv, w_o, w_pw1, dw, w_pw2, w_ff2a, w_ff2b,
):
    full = lambda a: pl.BlockSpec(a.shape, lambda b: (0,) * a.ndim)
    weights = (w_ff1a, w_ff1b, w_qkv, w_o, w_pw1, dw, w_pw2, w_ff2a, w_ff2b)
    u32 = lambda r, c: pltpu.VMEM((r // 2, c), U32)
    scratch = [
        u32(FF, D), u32(D, FF), u32(2 * D + H * VR, D), u32(D, H * VR), u32(2 * D, D), u32(D, D),
        u32(FF, D), u32(D, FF), pltpu.VMEM((KW, D, 128), F32),
        pltpu.VMEM((TP, D), BF16),
        pltpu.VMEM((D, TP), F32),
        pltpu.VMEM((H, KD // 2, TP), U32),
        pltpu.VMEM((2, TP // 2, KD), U32),
        pltpu.VMEM((H, VR, TP), F32),
        pltpu.VMEM((H, VR, TP), F32),
        pltpu.VMEM((D, TP + 256), F32),
        pltpu.VMEM((TP, D), BF16),
        pltpu.VMEM((TK, TQ), F32), pltpu.VMEM((TK, TQ), F32),
    ]
    return pl.pallas_call(
        _kernel,
        grid=(B,),
        in_specs=[pl.BlockSpec((1, T, D), lambda b: (b, 0, 0))] + [full(w) for w in weights],
        out_specs=pl.BlockSpec((1, T, D), lambda b: (b, 0, 0)),
        out_shape=jax.ShapeDtypeStruct((B, T, D), BF16),
        scratch_shapes=scratch,
        compiler_params=pltpu.CompilerParams(
            dimension_semantics=("arbitrary",), vmem_limit_bytes=100 * 1024 * 1024),
    )(x, *weights)
```

```python
import jax
import jax.numpy as jnp
import jax.experimental.pallas as pl
import jax.experimental.pallas.tpu as pltpu

F32 = jnp.float32
BF16 = jnp.bfloat16
U32 = jnp.uint32

B, T, D, H, DH, KW = 2, 4000, 144, 4, 36, 3
FF = 4 * D
TP = 4096
TB = 512
NB = TP // TB
NI = 4
TQ = 512
TK = 1024
RB = 128
VR = 40
HP = 2 * DH
KD = 128
EPS = 1e-5
NEG = -1e30
QSCALE = float(DH ** -0.5 * 1.4426950408889634)
CHUNKS = [(c * TK, min(TK, T - c * TK)) for c in range(-(-T // TK))]
NC = len(CHUNKS)
NSUB = [-(-size // RB) for _, size in CHUNKS]
LEAD = NSUB[0] + 1
NSB = 4
UPB = 4


def _pk(x):
    return pltpu.bitcast(x, U32)


def _upk(x):
    return pltpu.bitcast(x, BF16)


def _dot(a, b):
    return jnp.dot(a, b, preferred_element_type=F32)


def _ln(x):
    m = jnp.mean(x, axis=0, keepdims=True)
    xc = x - m
    v = jnp.mean(xc * xc, axis=0, keepdims=True)
    return xc * jax.lax.rsqrt(v + EPS)


def _silu_half(h):
    return h * jnp.tanh(h) + h


def _iota(shape, dim):
    return jax.lax.broadcasted_iota(jnp.int32, shape, dim)


def _kernel(x_hbm, w1a_ref, w1b_ref, wqkv_ref, wo_ref, wp1_ref, dw_ref, wp2_ref, w2a_ref, w2b_ref,
            o_hbm,
            x_ref, y_ref, x_sem, y_sem,
            w1a_t, w1b_t, wqkv_t, wo_t, wp1_t, wp2_t, w2a_t, w2b_t, dw_t,
            x1_ref, qt_ref, k_ref, vt_ref, acc_ref, g_ref, *S):
    b = pl.program_id(0)

    def x_copy(bb):
        return pltpu.make_async_copy(x_hbm.at[bb], x_ref.at[bb], x_sem.at[bb])

    def y_copy(bb, i):
        n = min(TB, T - i * TB)
        return pltpu.make_async_copy(y_ref.at[bb, :, i * TB:i * TB + n], o_hbm.at[bb, :, i * TB:i * TB + n],
                                     y_sem.at[bb * NB + i])

    @pl.when(b == 0)
    def _prep():
        for bb in range(B):
            x_copy(bb).start()
        tr = lambda w, scale=1.0: _pk((scale * w.astype(F32).T).astype(BF16))
        cp = lambda w, scale=1.0: _pk((scale * w.astype(F32)).astype(BF16))

        def pad_heads(w):
            zero = jnp.zeros((VR - DH, w.shape[1]), F32)
            return jnp.concatenate([p_ for h_ in range(H) for p_ in (w[h_ * DH:(h_ + 1) * DH], zero)], axis=0)

        w1a_t[...] = tr(w1a_ref[...], 0.5)
        w1b_t[...] = cp(w1b_ref[...], 0.5)
        w2a_t[...] = tr(w2a_ref[...], 0.5)
        w2b_t[...] = cp(w2b_ref[...], 0.5)
        wp1_t[...] = tr(wp1_ref[...], 0.5)
        wp2_t[...] = tr(wp2_ref[...])
        wqkv = wqkv_ref[...].astype(F32).T
        wqkv_t[...] = _pk(jnp.concatenate([wqkv[:2 * D], pad_heads(wqkv[2 * D:])], axis=0).astype(BF16))
        wo_t[...] = tr(pad_heads(wo_ref[...].astype(F32)))
        dwt = jnp.concatenate([0.5 * dw_ref[...].astype(F32), jnp.zeros((8 - KW, D), F32)], axis=0).T
        for i in range(KW):
            dw_t[i] = jnp.broadcast_to(dwt[:, i:i + 1], (D, 128))
        g_ref[:, 0:128] = jnp.zeros((D, 128), F32)
        g_ref[:, 128 + TP:] = jnp.zeros((D, 128), F32)

    x_copy(b).wait()

    def ffn(xs, wa_t, wb_t):
        hs = [_ln(x).astype(BF16) for x in xs]
        a_s = [_silu_half(_dot(_upk(wa_t[...]), h)).astype(BF16) for h in hs]
        return [x + _dot(_upk(wb_t[...]), a) for x, a in zip(xs, a_s)]

    def blocks(i):
        return [pl.multiple_of((i * NI + j) * TB, TB) for j in range(NI)]

    def phase1(i, carry):
        starts = blocks(i)
        xs = []
        for start in starts:
            tok = start + _iota((D, TB), 1)
            xs.append(jnp.where(tok < T, x_ref[b, :, pl.ds(start, TB)].astype(F32), 0.0))
        x1s = ffn(xs, w1a_t, w1b_t)
        for start, x1 in zip(starts, x1s):
            x1_ref[:, pl.ds(start, TB)] = x1
        hs = [_ln(x1).astype(BF16) for x1 in x1s]
        qkvs = [_dot(_upk(wqkv_t[...]), h) for h in hs]
        row = _iota((HP, TB), 0)
        vrow = _iota((H * VR, TB), 0)
        zpad = jnp.zeros((KD - HP, TB), F32)
        for start, qkv in zip(starts, qkvs):
            cols = pl.ds(start, TB)
            for pair in range(2):
                qp = qkv[pair * HP:(pair + 1) * HP] * QSCALE
                q_lo = jnp.concatenate([jnp.where(row < DH, qp, 0.0), zpad], axis=0)
                q_hi = jnp.concatenate([jnp.where(row >= DH, qp, 0.0), zpad], axis=0)
                qt_ref[2 * pair, :, cols] = _pk(q_lo.astype(BF16))
                qt_ref[2 * pair + 1, :, cols] = _pk(q_hi.astype(BF16))
                kt = jnp.concatenate([qkv[D + pair * HP:D + (pair + 1) * HP], zpad], axis=0)
                k_ref[pair, pl.ds(pl.multiple_of(start // 2, TB // 2), TB // 2), :] = _pk(kt.T.astype(BF16))
            v = jnp.where(vrow % VR == DH, 1.0, qkv[2 * D:])
            for h_ in range(H):
                vt_ref[h_, :, cols] = v[h_ * VR:(h_ + 1) * VR]
        return carry

    jax.lax.fori_loop(0, NB // NI, phase1, 0)

    NU = NB * H
    seq = [(j, c, r) for j in range(UPB) for c in range(NC) for r in range(NSUB[c])]

    def unit(u):
        u = jnp.minimum(u, NU - 1)
        return u // H, u % H

    def stage_a(u0, pos, z, mx):
        j, c, r = seq[pos % len(seq)]
        q, h = unit(u0 + j + (pos // len(seq)) * UPB)
        start, size = CHUNKS[c]
        n = min(RB, size - r * RB)
        off = (start + r * RB) // 2
        qt = _upk(qt_ref[h, :, pl.ds(pl.multiple_of(q * TQ, TQ), TQ)])
        k = _upk(k_ref[h // 2, off:off + n // 2, :])
        s = _dot(k, qt)
        S[c % NSB][pl.ds(pl.multiple_of(z + r * RB, 8), n), :] = s
        mr = jnp.max(s, axis=0, keepdims=True)
        key = (pos // len(seq), j, c)
        mx[key] = mr if r == 0 else jnp.maximum(mx[key], mr)

    def att_loop(i, carry):
        u0 = i * UPB
        z = (u0 // NU) * 8
        mx = {(0, 0, 0): carry[0], (0, 0, 1): carry[1]}
        for g, (j, c, r) in enumerate(seq):
            stage_a(u0, g + LEAD, z, mx)
            q, h = unit(u0 + j)
            start, size = CHUNKS[c]
            if r == 0:
                if c == 0:
                    m_new = mx[(0, j, c)]
                else:
                    m_prev = m_new
                    m_new = jnp.maximum(m_prev, mx[(0, j, c)])
                    alpha = jnp.exp2(m_prev - m_new)
            n = min(RB, size - r * RB)
            p = jnp.exp2(S[c % NSB][r * RB:r * RB + n, :] - m_new).astype(BF16)
            vt = vt_ref[h, :, start + r * RB:start + r * RB + n]
            d = _dot(vt, p)
            pv = d if r == 0 else pv + d
            if r == NSUB[c] - 1:
                acc = pv if c == 0 else acc * alpha + pv
                if c == NC - 1:
                    acc_ref[h, :, pl.ds(pl.multiple_of(q * TQ, TQ), TQ)] = acc
        return mx[(1, 0, 0)], mx[(1, 0, 1)]

    mx0 = {}
    for pos in range(LEAD):
        stage_a(0, pos, 0, mx0)
    jax.lax.fori_loop(0, NU // UPB, att_loop, (mx0[(0, 0, 0)], mx0[(0, 0, 1)]))

    rep = lambda w: jnp.concatenate([w] * (TB // 128), axis=1)
    x2, x3, x4, hh, cv, aa = {}, {}, {}, {}, {}, {}

    def st_wo(i):
        outs = []
        for h_ in range(H):
            a = acc_ref[h_, :, i * TB:(i + 1) * TB]
            outs.append(a * (1.0 / a[DH:DH + 1, :]))
        o = jnp.concatenate(outs, axis=0).astype(BF16)
        x2[i] = x1_ref[:, i * TB:(i + 1) * TB] + _dot(_upk(wo_t[...]), o)
        hh[1, i] = _ln(x2[i]).astype(BF16)

    def st_pw1(i):
        g = _dot(_upk(wp1_t[...]), hh.pop((1, i)))
        glu = g[:D] * jnp.tanh(g[D:]) + g[:D]
        if (i + 1) * TB > T:
            glu = jnp.where(i * TB + _iota((D, TB), 1) < T, glu, 0.0)
        g_ref[:, 128 + i * TB:128 + (i + 1) * TB] = glu

    def st_conv(i):
        win = g_ref[:, i * TB:(i + 1) * TB + 256]
        left = pltpu.roll(win, 1, 1)[:, 128:128 + TB]
        right = pltpu.roll(win, TB + 255, 1)[:, 128:128 + TB]
        cur = win[:, 128:128 + TB]
        c = left * rep(dw_t[0]) + cur * rep(dw_t[1]) + right * rep(dw_t[2])
        cv[i] = _silu_half(c).astype(BF16)

    def st_pw2(i):
        x3[i] = x2.pop(i) + _dot(_upk(wp2_t[...]), cv.pop(i))
        hh[2, i] = _ln(x3[i]).astype(BF16)

    def st_fa(i):
        aa[i] = _silu_half(_dot(_upk(w2a_t[...]), hh.pop((2, i)))).astype(BF16)

    def st_fb(i):
        x4[i] = x3.pop(i) + _dot(_upk(w2b_t[...]), aa.pop(i))

    def st_out(i):
        n = min(TB, T - i * TB)
        y_ref[b, :, i * TB:i * TB + n] = _ln(x4.pop(i)).astype(BF16)[:, :n]
        y_copy(b, i).start()

    ok = lambda i: 0 <= i < NB
    for k in range(-2, NB + 1):
        if ok(k):
            st_conv(k)
        if ok(k + 2):
            st_wo(k + 2)
        if ok(k - 1):
            st_fb(k - 1)
        if ok(k):
            st_pw2(k)
        if ok(k + 2):
            st_pw1(k + 2)
        if ok(k):
            st_fa(k)
        if ok(k - 1):
            st_out(k - 1)

    @pl.when(b == B - 1)
    def _drain():
        for bb in range(B):
            for i in range(NB):
                y_copy(bb, i).wait()


@jax.jit
def pallas_standalone__conformer_family_zipformer__speech_kernel(
    x, w_ff1a, w_ff1b, w_qkv, w_o, w_pw1, dw, w_pw2, w_ff2a, w_ff2b,
):
    full = lambda a: pl.BlockSpec(a.shape, lambda b: (0,) * a.ndim)
    weights = (w_ff1a, w_ff1b.T, w_qkv, w_o, w_pw1, dw, w_pw2, w_ff2a, w_ff2b.T)
    u32 = lambda r, c: pltpu.VMEM((r // 2, c), U32)
    scratch = [
        pltpu.VMEM((B, D, T), BF16), pltpu.VMEM((B, D, T), BF16),
        pltpu.SemaphoreType.DMA((B,)), pltpu.SemaphoreType.DMA((B * NB,)),
        u32(FF, D), u32(D, FF), u32(2 * D + H * VR, D), u32(D, H * VR), u32(2 * D, D), u32(D, D),
        u32(FF, D), u32(D, FF), pltpu.VMEM((KW, D, 128), F32),
        pltpu.VMEM((D, TP), F32),
        pltpu.VMEM((H, KD // 2, TP), U32),
        pltpu.VMEM((2, TP // 2, KD), U32),
        pltpu.VMEM((H, VR, TP), F32),
        pltpu.VMEM((H, VR, TP), F32),
        pltpu.VMEM((D, TP + 256), F32),
    ] + [pltpu.VMEM((TK, TQ), F32)] * NSB
    out_t = pl.pallas_call(
        _kernel,
        grid=(B,),
        in_specs=[pl.BlockSpec(memory_space=pl.ANY)] + [full(w) for w in weights],
        out_specs=pl.BlockSpec(memory_space=pl.ANY),
        out_shape=jax.ShapeDtypeStruct((B, D, T), BF16),
        scratch_shapes=scratch,
        compiler_params=pltpu.CompilerParams(
            dimension_semantics=("arbitrary",), vmem_limit_bytes=100 * 1024 * 1024),
    )(jnp.swapaxes(x, 1, 2), *weights)
    return jnp.swapaxes(out_t, 1, 2)
```

```python
import jax
import jax.numpy as jnp
import jax.experimental.pallas as pl
import jax.experimental.pallas.tpu as pltpu

F32 = jnp.float32
BF16 = jnp.bfloat16
U32 = jnp.uint32

B, T, D, H, DH, KW = 2, 4000, 144, 4, 36, 3
FF = 4 * D
TP = 4096
TB = 512
NB = TP // TB
NI = 4
TQ = 512
TK = 1024
RA = 256
RB = 128
VR = 40
HP = 2 * DH
KD = 128
QD = 80
EPS = 1e-5
QSCALE = float(DH ** -0.5 * 1.4426950408889634)
CHUNKS = [(c * TK, min(TK, T - c * TK)) for c in range(-(-T // TK))]
NC = len(CHUNKS)
NSB = NC
LEAD = TK // RA + 1
LAGW = 4


def _pk(x):
    return pltpu.bitcast(x, U32)


def _upk(x):
    return pltpu.bitcast(x, BF16)


def _dot(a, b):
    return jnp.dot(a, b, preferred_element_type=F32)


def _ln(x):
    m = jnp.mean(x, axis=0, keepdims=True)
    xc = x - m
    v = jnp.mean(xc * xc, axis=0, keepdims=True)
    return xc * jax.lax.rsqrt(v + EPS)


def _silu_half(h):
    return h * jnp.tanh(h) + h


def _iota(shape, dim):
    return jax.lax.broadcasted_iota(jnp.int32, shape, dim)


def _kernel(x_hbm, w1a_hbm, w1b_hbm, wqkv_hbm, wo_hbm, wp1_hbm, dw_hbm, wp2_hbm, w2a_hbm, w2b_hbm,
            o_hbm,
            x_ref, y_ref, x_sem, y_sem, w_sem,
            w1a_ref, w1b_ref, wqkv_ref, wo_ref, wp1_ref, dw_ref, wp2_ref, w2a_ref, w2b_ref,
            w1a_t, w1b_t, wqkv_t, wo_t, wp1_t, wp2_t, w2a_t, w2b_t, dw_t,
            x1_ref, qt_ref, k_ref, vt_ref, acc_ref, g_ref, *S):

    def x_copy(b):
        return pltpu.make_async_copy(x_hbm.at[b], x_ref.at[b], x_sem.at[b])

    def y_copy(b, i):
        n = min(TB, T - i * TB)
        return pltpu.make_async_copy(y_ref.at[b, :, i * TB:i * TB + n], o_hbm.at[b, :, i * TB:i * TB + n],
                                     y_sem.at[b * NB + i])

    w_pairs = ((w1a_hbm, w1a_ref), (w1b_hbm, w1b_ref), (wqkv_hbm, wqkv_ref), (w2a_hbm, w2a_ref),
               (w2b_hbm, w2b_ref), (wp1_hbm, wp1_ref), (wp2_hbm, wp2_ref), (wo_hbm, wo_ref),
               (dw_hbm, dw_ref))
    w_copies = [pltpu.make_async_copy(src, dst, w_sem.at[i]) for i, (src, dst) in enumerate(w_pairs)]
    for cp_ in w_copies:
        cp_.start()
    for b in range(B):
        x_copy(b).start()
    for cp_ in w_copies:
        cp_.wait()

    tr = lambda w, scale=1.0: _pk((scale * w.astype(F32).T).astype(BF16))
    cp = lambda w, scale=1.0: _pk((scale * w.astype(F32)).astype(BF16))

    def pad_heads(w):
        zero = jnp.zeros((VR - DH, w.shape[1]), F32)
        return jnp.concatenate([p_ for h in range(H) for p_ in (w[h * DH:(h + 1) * DH], zero)], axis=0)

    w1a_t[...] = tr(w1a_ref[...], 0.5)
    w1b_t[...] = cp(w1b_ref[...], 0.5)
    wqkv = wqkv_ref[...].astype(F32).T
    wqkv_t[...] = _pk(jnp.concatenate([wqkv[:2 * D], pad_heads(wqkv[2 * D:])], axis=0).astype(BF16))

    NG = NB // NI

    def phase1(it, carry):
        b = it // NG
        for bb in range(B):
            @pl.when(it == bb * NG)
            def _():
                x_copy(bb).wait()
        starts = [pl.multiple_of(((it % NG) * NI + j) * TB, TB) for j in range(NI)]
        xs = [jnp.where(start + _iota((D, TB), 1) < T, x_ref[b, :, pl.ds(start, TB)].astype(F32), 0.0)
              for start in starts]
        hs = [_ln(x).astype(BF16) for x in xs]
        acts = [_silu_half(_dot(_upk(w1a_t[...]), h)).astype(BF16) for h in hs]
        x1s = [x + _dot(_upk(w1b_t[...]), a) for x, a in zip(xs, acts)]
        for start, x1 in zip(starts, x1s):
            x1_ref[b, :, pl.ds(start, TB)] = x1
        hs = [_ln(x1).astype(BF16) for x1 in x1s]
        qkvs = [_dot(_upk(wqkv_t[...]), h) for h in hs]
        row = _iota((HP, TB), 0)
        vrow = _iota((H * VR, TB), 0)
        zpad = jnp.zeros((KD - HP, TB), F32)
        qpad = jnp.zeros((QD - HP, TB), F32)
        for start, qkv in zip(starts, qkvs):
            cols = pl.ds(start, TB)
            for pair in range(2):
                qp = qkv[pair * HP:(pair + 1) * HP] * QSCALE
                q_lo = jnp.concatenate([jnp.where(row < DH, qp, 0.0), qpad], axis=0)
                q_hi = jnp.concatenate([jnp.where(row >= DH, qp, 0.0), qpad], axis=0)
                qt_ref[b * H + 2 * pair, :, cols] = _pk(q_lo.astype(BF16))
                qt_ref[b * H + 2 * pair + 1, :, cols] = _pk(q_hi.astype(BF16))
                kt = jnp.concatenate([qkv[D + pair * HP:D + (pair + 1) * HP], zpad], axis=0)
                k_ref[b * 2 + pair, pl.ds(pl.multiple_of(start // 2, TB // 2), TB // 2), :] = (
                    _pk(kt.T.astype(BF16)))
            v = jnp.where(vrow % VR == DH, 1.0, qkv[2 * D:])
            for h in range(H):
                vt_ref[b * H + h, :, cols] = v[h * VR:(h + 1) * VR]
        return carry

    jax.lax.fori_loop(0, B * NG, phase1, 0)

    NBODY = B * NB
    seq_b = [(h, c, r) for h in range(H) for c in range(NC) for r in range(-(-CHUNKS[c][1] // RB))]
    seq_a = [(h, c, r) for h in range(H) for c in range(NC) for r in range(-(-CHUNKS[c][1] // RA))]

    def score(it, pos, z, mx):
        h, c, r = seq_a[pos % len(seq_a)]
        ahead = pos // len(seq_a)
        it = jnp.minimum(it + ahead, NBODY - 1)
        b, q = it // NB, it % NB
        start, size = CHUNKS[c]
        n = min(RA, size - r * RA)
        off = (start + r * RA) // 2
        qt = _upk(qt_ref[b * H + h, :, pl.ds(pl.multiple_of(q * TQ, TQ), TQ)])
        k = _upk(k_ref[b * 2 + h // 2, off:off + n // 2, 0:QD])
        s = _dot(k, qt)
        S[c % NSB][pl.ds(pl.multiple_of(z + r * RA, 8), n), :] = s
        mr = jnp.max(s, axis=0, keepdims=True)
        key = (ahead, h, c)
        mx[key] = mr if r == 0 else jnp.maximum(mx[key], mr)

    def attention(it, carry):
        b, q = it // NB, it % NB
        z = (it // NBODY) * 8
        mx = {(0, 0, 0): carry[0], (0, 0, 1): carry[1]}
        for g, (h, c, r) in enumerate(seq_b):
            if g % (RA // RB) == 0:
                score(it, g // (RA // RB) + LEAD, z, mx)
            start, size = CHUNKS[c]
            if r == 0:
                if c == 0:
                    m_new = mx[(0, h, c)]
                else:
                    m_prev = m_new
                    m_new = jnp.maximum(m_prev, mx[(0, h, c)])
                    alpha = jnp.exp2(m_prev - m_new)
            n = min(RB, size - r * RB)
            p = jnp.exp2(S[c % NSB][r * RB:r * RB + n, :] - m_new).astype(BF16)
            d = _dot(vt_ref[b * H + h, :, start + r * RB:start + r * RB + n], p)
            pv = d if r == 0 else pv + d
            if r * RB + n == size:
                acc = pv if c == 0 else acc * alpha + pv
                if c == NC - 1:
                    acc_ref[b * H + h, :, pl.ds(pl.multiple_of(q * TQ, TQ), TQ)] = acc
        return mx[(1, 0, 0)], mx[(1, 0, 1)]

    mx0 = {}
    for pos in range(LEAD):
        score(0, pos, 0, mx0)
    w2a_t[...] = tr(w2a_ref[...], 0.5)
    w2b_t[...] = cp(w2b_ref[...], 0.5)
    wp1_t[...] = tr(wp1_ref[...], 0.5)
    wp2_t[...] = tr(wp2_ref[...])
    wo_t[...] = tr(pad_heads(wo_ref[...].astype(F32)))
    dwt = jnp.concatenate([0.5 * dw_ref[...].astype(F32), jnp.zeros((8 - KW, D), F32)], axis=0).T
    for i in range(KW):
        dw_t[i] = jnp.broadcast_to(dwt[:, i:i + 1], (D, 128))
    g_ref[:, 0:128] = jnp.zeros((D, 128), F32)
    g_ref[:, 128 + TP:] = jnp.zeros((D, 128), F32)
    jax.lax.fori_loop(0, NBODY, attention, (mx0[(0, 0, 0)], mx0[(0, 0, 1)]))

    rep = lambda w: jnp.concatenate([w] * (TB // 128), axis=1)

    def phase3(b, carry):
        x2, x3, x4, hh, cv, aa = {}, {}, {}, {}, {}, {}

        def st_wo(i):
            outs = []
            for h in range(H):
                a = acc_ref[b * H + h, :, i * TB:(i + 1) * TB]
                outs.append(a * (1.0 / a[DH:DH + 1, :]))
            o = jnp.concatenate(outs, axis=0).astype(BF16)
            x2[i] = x1_ref[b, :, i * TB:(i + 1) * TB] + _dot(_upk(wo_t[...]), o)
            hh[1, i] = _ln(x2[i]).astype(BF16)

        def st_pw1(i):
            g = _dot(_upk(wp1_t[...]), hh.pop((1, i)))
            glu = g[:D] * jnp.tanh(g[D:]) + g[:D]
            if (i + 1) * TB > T:
                glu = jnp.where(i * TB + _iota((D, TB), 1) < T, glu, 0.0)
            g_ref[:, 128 + i * TB:128 + (i + 1) * TB] = glu

        def st_conv(i):
            win = g_ref[:, i * TB:(i + 1) * TB + 256]
            left = pltpu.roll(win, 1, 1)[:, 128:128 + TB]
            right = pltpu.roll(win, TB + 255, 1)[:, 128:128 + TB]
            cur = win[:, 128:128 + TB]
            c = left * rep(dw_t[0]) + cur * rep(dw_t[1]) + right * rep(dw_t[2])
            cv[i] = _silu_half(c).astype(BF16)

        def st_pw2(i):
            x3[i] = x2.pop(i) + _dot(_upk(wp2_t[...]), cv.pop(i))
            hh[2, i] = _ln(x3[i]).astype(BF16)

        def st_fa(i):
            aa[i] = _silu_half(_dot(_upk(w2a_t[...]), hh.pop((2, i)))).astype(BF16)

        def st_fb(i):
            x4[i] = x3.pop(i) + _dot(_upk(w2b_t[...]), aa.pop(i))

        def st_out(i):
            n = min(TB, T - i * TB)
            y_ref[b, :, i * TB:i * TB + n] = _ln(x4.pop(i)).astype(BF16)[:, :n]
            y_copy(b, i).start()

        for fn, idx in ((st_wo, 0), (st_wo, 1), (st_pw1, 0), (st_wo, 2), (st_pw1, 1), (st_wo, 3),
                        (st_pw1, 2), (st_pw1, 3)):
            fn(idx)
        for k in range(NB + 1):
            for fn, idx in ((st_conv, k), (st_pw2, k), (st_wo, k + LAGW), (st_fb, k - 1),
                            (st_pw1, k + LAGW), (st_fa, k), (st_out, k - 1)):
                if 0 <= idx < NB:
                    fn(idx)
        return carry

    jax.lax.fori_loop(0, B, phase3, 0)

    for b in range(B):
        for i in range(NB):
            y_copy(b, i).wait()


@jax.jit
def pallas_standalone__conformer_family_zipformer__speech_kernel(
    x, w_ff1a, w_ff1b, w_qkv, w_o, w_pw1, dw, w_pw2, w_ff2a, w_ff2b,
):
    weights = (w_ff1a, w_ff1b.T, w_qkv, w_o, w_pw1, dw, w_pw2, w_ff2a, w_ff2b.T)
    hbm = pl.BlockSpec(memory_space=pl.ANY)
    u32 = lambda r, c: pltpu.VMEM((r // 2, c), U32)
    scratch = [
        pltpu.VMEM((B, D, T), BF16), pltpu.VMEM((B, D, T), BF16),
        pltpu.SemaphoreType.DMA((B,)), pltpu.SemaphoreType.DMA((B * NB,)),
        pltpu.SemaphoreType.DMA((len(weights),)),
    ] + [pltpu.VMEM(w.shape, w.dtype) for w in weights] + [
        u32(FF, D), u32(D, FF), u32(2 * D + H * VR, D), u32(D, H * VR), u32(2 * D, D), u32(D, D),
        u32(FF, D), u32(D, FF), pltpu.VMEM((KW, D, 128), F32),
        pltpu.VMEM((B, D, TP), F32),
        pltpu.VMEM((B * H, QD // 2, TP), U32),
        pltpu.VMEM((B * 2, TP // 2, KD), U32),
        pltpu.VMEM((B * H, VR, TP), F32),
        pltpu.VMEM((B * H, VR, TP), F32),
        pltpu.VMEM((D, TP + 256), F32),
    ] + [pltpu.VMEM((TK, TQ), F32)] * NSB
    out_t = pl.pallas_call(
        _kernel,
        in_specs=[hbm] * (1 + len(weights)),
        out_specs=hbm,
        out_shape=jax.ShapeDtypeStruct((B, D, T), BF16),
        scratch_shapes=scratch,
        compiler_params=pltpu.CompilerParams(vmem_limit_bytes=100 * 1024 * 1024),
    )(jnp.swapaxes(x, 1, 2), *weights)
    return jnp.swapaxes(out_t, 1, 2)
```

```python
import jax
import jax.numpy as jnp
import jax.experimental.pallas as pl
import jax.experimental.pallas.tpu as pltpu

F32 = jnp.float32
BF16 = jnp.bfloat16
U32 = jnp.uint32

B, T, D, H, DH, KW = 2, 4000, 144, 4, 36, 3
FF = 4 * D
TP = 4096
TB = 512
NB = TP // TB
NI = 4
TQ = 512
TK = 256
RA = 256
RB = 128
VR = 40
HP = 2 * DH
KD = 128
QD = 80
EPS = 1e-5
QSCALE = float(DH ** -0.5 * 1.4426950408889634)
CHUNKS = [(c * TK, min(TK, T - c * TK)) for c in range(-(-T // TK))]
NC = len(CHUNKS)
NSB = 4
LEAD = TK // RA + 1
LAGW = 4


def _pk(x):
    return pltpu.bitcast(x, U32)


def _upk(x):
    return pltpu.bitcast(x, BF16)


def _dot(a, b):
    return jnp.dot(a, b, preferred_element_type=F32)


def _ln(x):
    m = jnp.mean(x, axis=0, keepdims=True)
    xc = x - m
    v = jnp.mean(xc * xc, axis=0, keepdims=True)
    return xc * jax.lax.rsqrt(v + EPS)


def _silu_half(h):
    return h * jnp.tanh(h) + h


def _iota(shape, dim):
    return jax.lax.broadcasted_iota(jnp.int32, shape, dim)


def _kernel(x_hbm, w1a_hbm, w1b_hbm, wqkv_hbm, wo_hbm, wp1_hbm, dw_hbm, wp2_hbm, w2a_hbm, w2b_hbm,
            o_hbm,
            x_ref, y_ref, x_sem, y_sem, w_sem,
            w1a_ref, w1b_ref, wqkv_ref, wo_ref, wp1_ref, dw_ref, wp2_ref, w2a_ref, w2b_ref,
            w1a_t, w1b_t, wqkv_t, wo_t, wp1_t, wp2_t, w2a_t, w2b_t, dw_t,
            x1_ref, qt_ref, k_ref, vt_ref, acc_ref, g_ref, *S):

    NG = NB // NI

    def x_copy(it):
        b, lo = it // NG, (it % NG) * NI * TB
        hi = min(lo + NI * TB, T)
        return pltpu.make_async_copy(x_hbm.at[b, :, lo:hi], x_ref.at[b, :, lo:hi], x_sem.at[it])

    def y_copy(b, i):
        n = min(TB, T - i * TB)
        return pltpu.make_async_copy(y_ref.at[b, :, i * TB:i * TB + n], o_hbm.at[b, :, i * TB:i * TB + n],
                                     y_sem.at[b * NB + i])

    w_pairs = ((w1a_hbm, w1a_ref), (w1b_hbm, w1b_ref), (wqkv_hbm, wqkv_ref), (w2a_hbm, w2a_ref),
               (w2b_hbm, w2b_ref), (wp1_hbm, wp1_ref), (wp2_hbm, wp2_ref), (wo_hbm, wo_ref),
               (dw_hbm, dw_ref))
    w_copies = [pltpu.make_async_copy(src, dst, w_sem.at[i]) for i, (src, dst) in enumerate(w_pairs)]
    for cp_ in w_copies[:3]:
        cp_.start()
    x_copy(0).start()
    for cp_ in w_copies[3:]:
        cp_.start()
    for it in range(1, B * NG):
        x_copy(it).start()
    for cp_ in w_copies[:3]:
        cp_.wait()

    tr = lambda w, scale=1.0: _pk((scale * w.astype(F32).T).astype(BF16))
    cp = lambda w, scale=1.0: _pk((scale * w.astype(F32)).astype(BF16))

    def pad_heads(w):
        zero = jnp.zeros((VR - DH, w.shape[1]), F32)
        return jnp.concatenate([p_ for h in range(H) for p_ in (w[h * DH:(h + 1) * DH], zero)], axis=0)

    w1a_t[...] = tr(w1a_ref[...], 0.5)
    w1b_t[...] = cp(w1b_ref[...], 0.5)
    wqkv = wqkv_ref[...].astype(F32).T
    wqkv_t[...] = _pk(jnp.concatenate([wqkv[:2 * D], pad_heads(wqkv[2 * D:])], axis=0).astype(BF16))

    def phase1(it, carry):
        b = it // NG
        for i_ in range(B * NG):
            @pl.when(it == i_)
            def _():
                x_copy(i_).wait()
        starts = [pl.multiple_of(((it % NG) * NI + j) * TB, TB) for j in range(NI)]
        xs = [jnp.where(start + _iota((D, TB), 1) < T, x_ref[b, :, pl.ds(start, TB)].astype(F32), 0.0)
              for start in starts]
        hs = [_ln(x).astype(BF16) for x in xs]
        acts = [_silu_half(_dot(_upk(w1a_t[...]), h)).astype(BF16) for h in hs]
        x1s = [x + _dot(_upk(w1b_t[...]), a) for x, a in zip(xs, acts)]
        for start, x1 in zip(starts, x1s):
            x1_ref[b, :, pl.ds(start, TB)] = x1
        hs = [_ln(x1).astype(BF16) for x1 in x1s]
        qkvs = [_dot(_upk(wqkv_t[...]), h) for h in hs]
        row = _iota((HP, TB), 0)
        vrow = _iota((H * VR, TB), 0)
        zpad = jnp.zeros((KD - HP, TB), F32)
        qpad = jnp.zeros((QD - HP, TB), F32)
        for start, qkv in zip(starts, qkvs):
            cols = pl.ds(start, TB)
            for pair in range(2):
                qp = qkv[pair * HP:(pair + 1) * HP] * QSCALE
                q_lo = jnp.concatenate([jnp.where(row < DH, qp, 0.0), qpad], axis=0)
                q_hi = jnp.concatenate([jnp.where(row >= DH, qp, 0.0), qpad], axis=0)
                qt_ref[b * H + 2 * pair, :, cols] = _pk(q_lo.astype(BF16))
                qt_ref[b * H + 2 * pair + 1, :, cols] = _pk(q_hi.astype(BF16))
                kt = jnp.concatenate([qkv[D + pair * HP:D + (pair + 1) * HP], zpad], axis=0)
                k_ref[b * 2 + pair, pl.ds(pl.multiple_of(start // 2, TB // 2), TB // 2), :] = (
                    _pk(kt.T.astype(BF16)))
            v = jnp.where(vrow % VR == DH, 1.0, qkv[2 * D:])
            for h in range(H):
                vt_ref[b * H + h, :, cols] = v[h * VR:(h + 1) * VR]
        return carry

    jax.lax.fori_loop(0, B * NG, phase1, 0)

    NBODY = B * NB
    seq_b = [(h, c, r) for h in range(H) for c in range(NC) for r in range(-(-CHUNKS[c][1] // RB))]
    seq_a = [(h, c, r) for h in range(H) for c in range(NC) for r in range(-(-CHUNKS[c][1] // RA))]

    def score(it, pos, z, mx):
        h, c, r = seq_a[pos % len(seq_a)]
        ahead = pos // len(seq_a)
        it = jnp.minimum(it + ahead, NBODY - 1)
        b, q = it // NB, it % NB
        start, size = CHUNKS[c]
        n = min(RA, size - r * RA)
        off = (start + r * RA) // 2
        qt = _upk(qt_ref[b * H + h, :, pl.ds(pl.multiple_of(q * TQ, TQ), TQ)])
        k = _upk(k_ref[b * 2 + h // 2, off:off + n // 2, 0:QD])
        s = _dot(k, qt)
        S[c % NSB][pl.ds(pl.multiple_of(z + r * RA, 8), n), :] = s
        mr = jnp.max(s, axis=0, keepdims=True)
        key = (ahead, h, c)
        mx[key] = mr if r == 0 else jnp.maximum(mx[key], mr)

    def attention(it, carry):
        b, q = it // NB, it % NB
        z = (it // NBODY) * 8
        mx = {(0, 0, 0): carry[0], (0, 0, 1): carry[1]}
        for g, (h, c, r) in enumerate(seq_b):
            if g % (RA // RB) == 0:
                score(it, g // (RA // RB) + LEAD, z, mx)
            start, size = CHUNKS[c]
            if r == 0:
                if c == 0:
                    m_new = mx[(0, h, c)]
                else:
                    m_prev = m_new
                    m_new = jnp.maximum(m_prev, mx[(0, h, c)])
                    alpha = jnp.exp2(m_prev - m_new)
            n = min(RB, size - r * RB)
            p = jnp.exp2(S[c % NSB][r * RB:r * RB + n, :] - m_new).astype(BF16)
            d = _dot(vt_ref[b * H + h, :, start + r * RB:start + r * RB + n], p)
            pv = d if r == 0 else pv + d
            if r * RB + n == size:
                acc = pv if c == 0 else acc * alpha + pv
                if c == NC - 1:
                    acc_ref[b * H + h, :, pl.ds(pl.multiple_of(q * TQ, TQ), TQ)] = acc
        return mx[(1, 0, 0)], mx[(1, 0, 1)]

    for cp_ in w_copies[3:]:
        cp_.wait()
    mx0 = {}
    for pos in range(LEAD):
        score(0, pos, 0, mx0)
    w2a_t[...] = tr(w2a_ref[...], 0.5)
    w2b_t[...] = cp(w2b_ref[...], 0.5)
    wp1_t[...] = tr(wp1_ref[...], 0.5)
    wp2_t[...] = tr(wp2_ref[...])
    wo_t[...] = tr(pad_heads(wo_ref[...].astype(F32)))
    dwt = jnp.concatenate([0.5 * dw_ref[...].astype(F32), jnp.zeros((8 - KW, D), F32)], axis=0).T
    for i in range(KW):
        dw_t[i] = jnp.broadcast_to(dwt[:, i:i + 1], (D, 128))
    g_ref[:, 0:128] = jnp.zeros((D, 128), F32)
    g_ref[:, 128 + TP:] = jnp.zeros((D, 128), F32)
    jax.lax.fori_loop(0, NBODY, attention, (mx0[(0, 0, 0)], mx0[(0, 0, 1)]))

    rep = lambda w: jnp.concatenate([w] * (TB // 128), axis=1)

    def phase3(b, carry):
        x2, x3, x4, hh, cv, aa = {}, {}, {}, {}, {}, {}

        def st_wo(i):
            outs = []
            for h in range(H):
                a = acc_ref[b * H + h, :, i * TB:(i + 1) * TB]
                outs.append(a * (1.0 / a[DH:DH + 1, :]))
            o = jnp.concatenate(outs, axis=0).astype(BF16)
            x2[i] = x1_ref[b, :, i * TB:(i + 1) * TB] + _dot(_upk(wo_t[...]), o)
            hh[1, i] = _ln(x2[i]).astype(BF16)

        def st_pw1(i):
            g = _dot(_upk(wp1_t[...]), hh.pop((1, i)))
            glu = g[:D] * jnp.tanh(g[D:]) + g[:D]
            if (i + 1) * TB > T:
                glu = jnp.where(i * TB + _iota((D, TB), 1) < T, glu, 0.0)
            g_ref[:, 128 + i * TB:128 + (i + 1) * TB] = glu

        def st_conv(i):
            win = g_ref[:, i * TB:(i + 1) * TB + 256]
            left = pltpu.roll(win, 1, 1)[:, 128:128 + TB]
            right = pltpu.roll(win, TB + 255, 1)[:, 128:128 + TB]
            cur = win[:, 128:128 + TB]
            c = left * rep(dw_t[0]) + cur * rep(dw_t[1]) + right * rep(dw_t[2])
            cv[i] = _silu_half(c).astype(BF16)

        def st_pw2(i):
            x3[i] = x2.pop(i) + _dot(_upk(wp2_t[...]), cv.pop(i))
            hh[2, i] = _ln(x3[i]).astype(BF16)

        def st_fa(i):
            aa[i] = _silu_half(_dot(_upk(w2a_t[...]), hh.pop((2, i)))).astype(BF16)

        def st_fb(i):
            x4[i] = x3.pop(i) + _dot(_upk(w2b_t[...]), aa.pop(i))

        def st_out(i):
            n = min(TB, T - i * TB)
            y_ref[b, :, i * TB:i * TB + n] = _ln(x4.pop(i)).astype(BF16)[:, :n]
            y_copy(b, i).start()

        for fn, idx in ((st_wo, 0), (st_wo, 1), (st_pw1, 0), (st_wo, 2), (st_pw1, 1), (st_wo, 3),
                        (st_pw1, 2), (st_pw1, 3)):
            fn(idx)
        for k in range(NB + 1):
            for fn, idx in ((st_conv, k), (st_pw2, k), (st_wo, k + LAGW), (st_fb, k - 1),
                            (st_pw1, k + LAGW), (st_fa, k), (st_out, k - 1)):
                if 0 <= idx < NB:
                    fn(idx)
        return carry

    jax.lax.fori_loop(0, B, phase3, 0)

    for b in range(B):
        for i in range(NB):
            y_copy(b, i).wait()


@jax.jit
def pallas_standalone__conformer_family_zipformer__speech_kernel(
    x, w_ff1a, w_ff1b, w_qkv, w_o, w_pw1, dw, w_pw2, w_ff2a, w_ff2b,
):
    weights = (w_ff1a, w_ff1b.T, w_qkv, w_o, w_pw1, dw, w_pw2, w_ff2a, w_ff2b.T)
    hbm = pl.BlockSpec(memory_space=pl.ANY)
    u32 = lambda r, c: pltpu.VMEM((r // 2, c), U32)
    scratch = [
        pltpu.VMEM((B, D, T), BF16), pltpu.VMEM((B, D, T), BF16),
        pltpu.SemaphoreType.DMA((B * NB // NI,)), pltpu.SemaphoreType.DMA((B * NB,)),
        pltpu.SemaphoreType.DMA((len(weights),)),
    ] + [pltpu.VMEM(w.shape, w.dtype) for w in weights] + [
        u32(FF, D), u32(D, FF), u32(2 * D + H * VR, D), u32(D, H * VR), u32(2 * D, D), u32(D, D),
        u32(FF, D), u32(D, FF), pltpu.VMEM((KW, D, 128), F32),
        pltpu.VMEM((B, D, TP), F32),
        pltpu.VMEM((B * H, QD // 2, TP), U32),
        pltpu.VMEM((B * 2, TP // 2, KD), U32),
        pltpu.VMEM((B * H, VR, TP), F32),
        pltpu.VMEM((B * H, VR, TP), F32),
        pltpu.VMEM((D, TP + 256), F32),
    ] + [pltpu.VMEM((TK, TQ), F32)] * NSB
    out_t = pl.pallas_call(
        _kernel,
        in_specs=[hbm] * (1 + len(weights)),
        out_specs=hbm,
        out_shape=jax.ShapeDtypeStruct((B, D, T), BF16),
        scratch_shapes=scratch,
        compiler_params=pltpu.CompilerParams(vmem_limit_bytes=100 * 1024 * 1024),
    )(jnp.swapaxes(x, 1, 2), *weights)
    return jnp.swapaxes(out_t, 1, 2)
```
